```python
import jax
import jax.numpy as jnp

def _softmax(x, axis=-1):
    return jax.nn.softmax(x, axis=axis)
def _gelu(x):
    return jax.nn.gelu(x, approximate=True)
def _silu(x):
    return jax.nn.silu(x)
def _sigmoid(x):
    return jax.nn.sigmoid(x)
def _layernorm(x, axis=-1, eps=1e-5):
    m = jnp.mean(x, axis=axis, keepdims=True)
    v = jnp.var(x, axis=axis, keepdims=True)
    return (x - m) / jnp.sqrt(v + eps)
def _scatter_add(tgt, idx, src, axis=0):
    return tgt.at[idx].add(src)
def _segment_sum(src, seg, n):
    return jax.ops.segment_sum(src, seg, n)
class _Rng:
    def __init__(self, key):
        self._k = key
    def _next(self):
        self._k, sub = jax.random.split(self._k)
        return sub
    def normal(self, shape):
        return jax.random.normal(self._next(), shape, dtype=jnp.bfloat16)
    def randint(self, lo, hi, shape):
        return jax.random.randint(self._next(), shape, lo, hi, dtype=jnp.int32)
    def uniform(self, shape, lo=0.0, hi=1.0):
        return jax.random.uniform(self._next(), shape, jnp.bfloat16, lo, hi)
    def permutation(self, n):
        return jax.random.permutation(self._next(), n)


kernel_name = 'concat_heads__gqa_block_cached__compressed_kv_cla__decode'

def setup_inputs():
    _rng = _Rng(jax.random.key(int.from_bytes(__import__("os").urandom(4), "little")))
    _w = (lambda a: (lambda t: t.astype(jnp.bfloat16) if jnp.issubdtype(t.dtype, jnp.floating) else t)(jnp.asarray(a)))
    def _A_setup():
        B, Sq, D = 2, 1, 512
        Hq, Hkv, Sk, Dh = 32, 32, 8192, 128
        assert Hq % Hkv == 0, (Hq, Hkv)
        return {
            "x": _w((lambda *s: _rng.normal(s) * 0.05)(B, Sq, D)),
            "k_cache": _w((lambda *s: _rng.normal(s) * 0.05)(B, Hkv, Sk, Dh)),
            "v_cache": _w((lambda *s: _rng.normal(s) * 0.05)(B, Hkv, Sk, Dh)),
            "wq": _w((lambda *s: _rng.normal(s) * 0.05)(D, Hq * Dh) * (D ** -0.5)),
            "wo": _w((lambda *s: _rng.normal(s) * 0.05)(Hq * Dh, D) * ((Hq * Dh) ** -0.5)),
        }
    _A_in = _A_setup()

    def _B_setup():
        B, H, Sq, Sk, D, M = 2, 32, 1, 8192, 128, 512
        Dc = 4 * D
        return {
            "x": _w((lambda *s: _rng.normal(s) * 0.05)(B, Sq, M)),
            "c_kv": _w((lambda *s: _rng.normal(s) * 0.05)(B, Sk, Dc)),
            "w_q": _w((lambda *s: _rng.normal(s) * 0.05)(M, H, D) * (M ** -0.5)),
            "w_uk": _w((lambda *s: _rng.normal(s) * 0.05)(Dc, H, D) * (Dc ** -0.5)),
            "w_uv": _w((lambda *s: _rng.normal(s) * 0.05)(Dc, H, D) * (Dc ** -0.5)),
            "w_o": _w((lambda *s: _rng.normal(s) * 0.05)(H, D, M) * ((H * D) ** -0.5)),
        }
    _B_in = _B_setup()

    return {
        "A_x": _A_in["x"],
        "A_k_cache": _A_in["k_cache"],
        "A_v_cache": _A_in["v_cache"],
        "A_wq": _A_in["wq"],
        "A_wo": _A_in["wo"],
        "B_x": _B_in["x"],
        "B_c_kv": _B_in["c_kv"],
        "B_w_q": _B_in["w_q"],
        "B_w_uk": _B_in["w_uk"],
        "B_w_uv": _B_in["w_uv"],
        "B_w_o": _B_in["w_o"],
    }

def reference(A_x, A_k_cache, A_v_cache, A_wq, A_wo, B_x, B_c_kv, B_w_q, B_w_uk, B_w_uv, B_w_o):
    def _A_ref(x, k_cache, v_cache, wq, wo):
        B, Sq, D = x.shape
        Hq, Dh = 32, 128
        Hkv = k_cache.shape[1]
        rep = Hq // Hkv
        q = (lambda x, *d: x.transpose(*d))((x @ wq).reshape(B, Sq, Hq, Dh), 0, 2, 1, 3)
        k = jnp.repeat(k_cache, rep, axis=1)
        v = jnp.repeat(v_cache, rep, axis=1)
        scores = jnp.einsum("bhqd,bhkd->bhqk", q, k) * (Dh ** -0.5)
        p = _softmax(scores, axis=-1)
        o = jnp.einsum("bhqk,bhkd->bhqd", p, v)
        return (lambda x, *d: x.transpose(*d))(o, 0, 2, 1, 3).reshape(B, Sq, Hq * Dh) @ wo

    def _B_ref(x, c_kv, w_q, w_uk, w_uv, w_o):
        B, Sq, M = x.shape[0], x.shape[1], x.shape[2]
        Sk = c_kv.shape[1]
        H, D = w_q.shape[1], w_q.shape[2]
        q = jnp.einsum("bqm,mhd->bhqd", x, w_q)
        k = jnp.einsum("bkc,chd->bhkd", c_kv, w_uk)
        v = jnp.einsum("bkc,chd->bhkd", c_kv, w_uv)
        scores = jnp.einsum("bhqd,bhkd->bhqk", q, k) * (D ** -0.5)
        off = Sk - Sq
        qi = jnp.arange(Sq)[:, None]
        kj = jnp.arange(Sk)[None, :]
        cmask = kj <= (qi + off)
        scores = jnp.where(cmask[None, None], scores, -1e9)
        p = _softmax(scores, axis=-1)
        ctx = jnp.einsum("bhqk,bhkd->bhqd", p, v)
        return jnp.einsum("bhqd,hdm->bqm", ctx, w_o)

    a = _A_ref(A_x, A_k_cache, A_v_cache, A_wq, A_wo)
    b = _B_ref(B_x, B_c_kv, B_w_q, B_w_uk, B_w_uv, B_w_o)
    return jnp.concatenate([a, b], axis=-1)
```

```python
import functools
import numpy as np
import jax
import jax.numpy as jnp
from jax import lax
import jax.experimental.pallas as pl
import jax.experimental.pallas.tpu as pltpu

BF = jnp.bfloat16
F32 = jnp.float32
NT = (((1,), (1,)), ((), ()))


def _split_pair(w32):
    lo = pltpu.bitcast(w32 << 16, F32).astype(BF)
    hi = pltpu.bitcast(w32 & jnp.uint32(0xFFFF0000), F32).astype(BF)
    return lo, hi


def make_kernel(CH=2048, NSLOT=4, D=3, CB=1024, prio=False):
    NB, H, S, DH, M, DC = 2, 32, 8192, 128, 512, 512
    NC = S // CH
    NCH = 2 * NC
    assert NCH % NSLOT == 0 and D <= NSLOT - 1
    NCB = NB * S // CB
    scale = float(DH) ** -0.5

    def kernel(xa_h, k_h, v_h, wq_h, wo_h, xb_h, c_h, wbq_h, wuk_h, wuv_h, wbo_h,
               out_ref,
               xa_s, xb_s, wq_s, wo_s, c_s, wbq_s, wuk_s, wuv_s, wbo_s,
               ring, q_s, s_s, lat_s, ctx_s, sem_w, sem_c, sem_kv):
        row8 = lambda n: lax.broadcasted_iota(jnp.int32, (8, n), 0)

        cp_xa = pltpu.make_async_copy(xa_h, xa_s, sem_w.at[0])
        cp_xb = pltpu.make_async_copy(xb_h, xb_s, sem_w.at[1])
        cp_wbq = pltpu.make_async_copy(wbq_h, wbq_s, sem_w.at[2])
        cp_wuk = pltpu.make_async_copy(wuk_h, wuk_s, sem_w.at[3])
        cp_wuv = pltpu.make_async_copy(wuv_h, wuv_s, sem_w.at[4])
        cp_wbo = pltpu.make_async_copy(wbo_h, wbo_s, sem_w.at[5])
        cp_wq = pltpu.make_async_copy(wq_h, wq_s, sem_w.at[6])
        cp_wo = pltpu.make_async_copy(wo_h, wo_s, sem_w.at[7])

        def cp_c(j):
            return pltpu.make_async_copy(c_h.at[pl.ds(j * CB, CB), :], c_s.at[pl.ds(j * CB, CB), :], sem_c.at[j])

        def cp_kv(head, r):
            slot = r % NSLOT
            if r < NC:
                src = k_h.at[head, pl.ds(r * CH, CH), :]
            else:
                src = v_h.at[head, pl.ds((r - NC) * CH, CH), :]
            return pltpu.make_async_copy(src, ring.at[slot], sem_kv.at[slot])

        cp_xb.start()
        cp_xa.start()
        cp_wbq.start()
        cp_wuk.start()

        def pad_rows(x2):
            n = x2.shape[1]
            r = row8(n)
            return jnp.where(r == 0, x2[0:1, :], jnp.where(r == 1, x2[1:2, :], 0.0))

        cp_xb.wait()
        xb8 = pad_rows(xb_s[...].astype(F32)).astype(BF)
        cp_wbq.wait()
        cp_wuk.wait()
        for j in range(4):
            cp_c(j).start()

        wbq32 = wbq_s.bitcast(jnp.uint32)
        wuk32 = wuk_s.bitcast(jnp.uint32)

        def qlat_body(i, carry):
            wq_pair = _split_pair(wbq32[pl.ds(i, M, stride=H // 2), :])
            wk_pair = _split_pair(wuk32[pl.ds(i, DC, stride=H // 2), :])
            for e in range(2):
                q = jnp.dot(xb8, wq_pair[e], preferred_element_type=F32).astype(BF)
                ql = lax.dot_general(q, wk_pair[e], NT, preferred_element_type=F32)
                for b in range(NB):
                    lat_s[b, pl.ds(2 * i + e, 1), :] = ql[b:b + 1, :]
            return carry
        for i in range(H // 2):
            qlat_body(i, 0)

        for b in range(NB):
            ql = lat_s[b].astype(BF)
            m = jnp.full((H, 1), -jnp.inf, F32)
            l = jnp.zeros((H, 1), F32)
            acc = jnp.zeros((H, DC), F32)
            for jj in range(S // CB):
                j = b * (S // CB) + jj
                cp_c(j).wait()
                nxt = j + 4
                if nxt < NCB:
                    cp_c(nxt).start()
                elif nxt == NCB:
                    cp_wuv.start()
                elif nxt == NCB + 1:
                    cp_wbo.start()
                elif nxt == NCB + 2:
                    cp_wq.start()
                elif nxt == NCB + 3:
                    cp_wo.start()
                cc = c_s[pl.ds(j * CB, CB), :]
                s = lax.dot_general(ql, cc, NT, preferred_element_type=F32) * scale
                m_new = jnp.maximum(m, jnp.max(s, axis=1, keepdims=True))
                alpha = jnp.exp(m - m_new)
                p = jnp.exp(s - m_new)
                l = alpha * l + jnp.sum(p, axis=1, keepdims=True)
                acc = alpha * acc + jnp.dot(p.astype(BF), cc, preferred_element_type=F32)
                m = m_new
            ctx_s[b] = acc / l

        for r in range(D):
            cp_kv(0, r).start()

        cp_wuv.wait()
        cp_wbo.wait()
        wuv32 = wuv_s.bitcast(jnp.uint32)
        out_b = jnp.zeros((8, M), F32)
        r512 = row8(DC)
        for i in range(H // 2):
            wv_pair = _split_pair(wuv32[pl.ds(i, DC, stride=H // 2), :])
            for e in range(2):
                h = 2 * i + e
                c0 = ctx_s[0, pl.ds(h, 1), :]
                c1 = ctx_s[1, pl.ds(h, 1), :]
                lhs = jnp.where(r512 == 0, c0, jnp.where(r512 == 1, c1, 0.0)).astype(BF)
                ctx = jnp.dot(lhs, wv_pair[e], preferred_element_type=F32).astype(BF)
                out_b = out_b + jnp.dot(ctx, wbo_s[h], preferred_element_type=F32)

        cp_xa.wait()
        xa8 = pad_rows(xa_s[...].astype(F32)).astype(BF)
        cp_wq.wait()
        qa = jnp.dot(xa8, wq_s[...], preferred_element_type=F32).astype(BF)
        for h in range(H):
            q_s[h] = qa[:, h * DH:(h + 1) * DH]
        cp_wo.wait()

        r128 = row8(DH)

        def head_body(i, out_a):
            b = i // H
            h = i % H
            q = q_s[h]
            mx = jnp.full((8, DH), -jnp.inf, F32)
            acc = jnp.zeros((8, DH), F32)
            lsum = jnp.zeros((8, DH), F32)
            for r in range(NCH):
                cp_kv(i, r).wait()
                nr = r + D
                if nr < NCH:
                    cp_kv(i, nr).start()
                else:
                    @pl.when(i + 1 < NB * H)
                    def _():
                        cp_kv(i + 1, nr - NCH).start()
                buf = ring[r % NSLOT]
                if r < NC:
                    s = lax.dot_general(q, buf, NT, preferred_element_type=F32)
                    s_s[:, r * CH:(r + 1) * CH] = s
                    for t in range(CH // DH):
                        mx = jnp.maximum(mx, s[:, t * DH:(t + 1) * DH])
                    if r == NC - 1:
                        mrow = jnp.max(mx, axis=1, keepdims=True)
                else:
                    rr = r - NC
                    p = jnp.exp((s_s[:, rr * CH:(rr + 1) * CH] - mrow) * scale)
                    for t in range(CH // DH):
                        lsum = lsum + p[:, t * DH:(t + 1) * DH]
                    acc = acc + jnp.dot(p.astype(BF), buf, preferred_element_type=F32)
            l = jnp.sum(lsum, axis=1, keepdims=True)
            o = jnp.where(r128 == b, acc / l, 0.0).astype(BF)
            return out_a + jnp.dot(o, wo_s[h], preferred_element_type=F32)

        out_a = lax.fori_loop(0, NB * H, head_body, jnp.zeros((8, M), F32))
        out_ref[:, 0:M] = out_a[0:2, :].astype(out_ref.dtype)
        out_ref[:, M:2 * M] = out_b[0:2, :].astype(out_ref.dtype)

    @jax.jit
    def fn(A_x, A_k_cache, A_v_cache, A_wq, A_wo, B_x, B_c_kv, B_w_q, B_w_uk, B_w_uv, B_w_o):
        args = (
            A_x.reshape(NB, M),
            A_k_cache.reshape(NB * H, S, DH),
            A_v_cache.reshape(NB * H, S, DH),
            A_wq,
            A_wo.reshape(H, DH, M),
            B_x.reshape(NB, M),
            B_c_kv.reshape(NB * S, DC),
            B_w_q.reshape(M * H, DH),
            B_w_uk.reshape(DC * H, DH),
            B_w_uv.reshape(DC * H, DH),
            B_w_o,
        )
        out = pl.pallas_call(
            kernel,
            in_specs=[pl.BlockSpec(memory_space=pl.ANY)] * 11,
            out_specs=pl.BlockSpec(memory_space=pltpu.VMEM),
            out_shape=jax.ShapeDtypeStruct((NB, 2 * M), BF),
            scratch_shapes=[
                pltpu.VMEM((NB, M), BF), pltpu.VMEM((NB, M), BF),
                pltpu.VMEM((M, H * DH), BF), pltpu.VMEM((H, DH, M), BF),
                pltpu.VMEM((NB * S, DC), BF),
                pltpu.VMEM((M * H, DH), BF), pltpu.VMEM((DC * H, DH), BF), pltpu.VMEM((DC * H, DH), BF),
                pltpu.VMEM((H, DH, M), BF),
                pltpu.VMEM((NSLOT, CH, DH), BF),
                pltpu.VMEM((H, 8, DH), BF),
                pltpu.VMEM((8, S), F32),
                pltpu.VMEM((NB, H, DC), F32),
                pltpu.VMEM((NB, H, DC), F32),
                pltpu.SemaphoreType.DMA((8,)),
                pltpu.SemaphoreType.DMA((NCB,)),
                pltpu.SemaphoreType.DMA((NSLOT,)),
            ],
            compiler_params=pltpu.CompilerParams(vmem_limit_bytes=100 * 1024 * 1024),
        )(*args)
        return out.reshape(NB, 1, 2 * M)
    return fn


_impl = make_kernel()


@jax.jit
def pallas_concat_heads__gqa_block_cached__compressed_kv_cla__decode_kernel(
    A_x: jax.Array,
    A_k_cache: jax.Array,
    A_v_cache: jax.Array,
    A_wq: jax.Array,
    A_wo: jax.Array,
    B_x: jax.Array,
    B_c_kv: jax.Array,
    B_w_q: jax.Array,
    B_w_uk: jax.Array,
    B_w_uv: jax.Array,
    B_w_o: jax.Array,
):
    return _impl(A_x, A_k_cache, A_v_cache, A_wq, A_wo,
                 B_x, B_c_kv, B_w_q, B_w_uk, B_w_uv, B_w_o)
```

```python
import contextlib
import numpy as np
import jax
import jax.numpy as jnp
from jax import lax
import jax.experimental.pallas as pl
import jax.experimental.pallas.tpu as pltpu

BF = jnp.bfloat16
F32 = jnp.float32
U32 = jnp.uint32
NT = (((1,), (1,)), ((), ()))

NB, H, S, DH, M, DC = 2, 32, 8192, 128, 512, 512
G = 8
TR = 128
NSG = 8
NSTEP = S // TR
NGRP = NB * H // G
NK = NGRP * NSTEP


def _halves(w32):
    lo = pltpu.bitcast(w32 << 16, F32).astype(BF)
    hi = pltpu.bitcast(w32 & jnp.uint32(0xFFFF0000), F32).astype(BF)
    return lo, hi


def make_kernel(L=6, comp=True, scopes=False, pk=0, pv=1, cparams=None, skip=(), EW=2, EP=4):
    scale = float(DH) ** -0.5
    cparams = cparams or {}

    def scope(name):
        return jax.named_scope(name) if scopes else contextlib.nullcontext()

    E_WO, E_W0, E_W1, E_C, E_END = 0, 8, 24, 40, 72
    P_T1, P_T3 = 24, 72

    def kernel(xa_h, k_h, v_h, wq_h, wo_h, xb_h, c_h, wbq_h, wuk_h, wuv_h, wbo_h,
               out_ref,
               xa_s, xb_s, wq_s, wo_s, c_s, wbq_s, wuk_s, wuv_s, wbo_s,
               kv_s, q_s, lat_s, lm_s, ll_s, lacc_s, ob_s, oa_s, sem_x, sem_q, sem_e, sem_kv):

        cp = pltpu.make_async_copy

        def start_pairs(pairs):
            for a, b in pairs:
                a.start(priority=pk)
                b.start(priority=pv)

        def head_w(src, dst, j, d, sem):
            rows = pl.ds(pl.multiple_of((j * 8 + d) * 32, 32), 32)
            return cp(src.at[:, rows, :], dst.at[:, rows, :], sem)

        def head_w_all(dst, j, sem):
            v = dst.at[:, pl.ds(pl.multiple_of(j * 256, 256), 256), :]
            return cp(v, v, sem)

        def out_w(src, dst, r16, ch, sem):
            rows = pl.ds(pl.multiple_of(r16 * 16, 16), 16)
            cols = pl.ds(ch * 256, 256)
            return cp(src.at[:, rows, cols], dst.at[:, rows, cols], sem)

        def rows_all(dst, r0, n, sem):
            v = dst.at[:, pl.ds(r0, n), :]
            return cp(v, v, sem)

        def start_q(j):
            rows = pl.ds(j * 16, 16)
            def one(d):
                cols = pl.ds(d * 256, 256)
                return cp(wq_h.at[:, rows, cols], wq_s.at[:, rows, cols], sem_q.at[j])
            start_pairs([(one(2 * d), one(2 * d + 1)) for d in range(8)])

        def wait_q(j):
            v = wq_s.at[:, pl.ds(j * 16, 16), :]
            cp(v, v, sem_q.at[j]).wait()

        def start_extra(e):
            sem = sem_e.at[e & 3]

            @pl.when(e < E_W0)
            def _():
                j = e - E_WO
                start_pairs([(out_w(wo_h, wo_s, j * 8 + d, 0, sem), out_w(wo_h, wo_s, j * 8 + d, 1, sem))
                             for d in range(8)])

            @pl.when((e >= E_W0) & (e < E_W1))
            def _():
                j = e - E_W0
                start_pairs([(head_w(wbq_h, wbq_s, j, d, sem), head_w(wuk_h, wuk_s, j, d, sem)) for d in range(8)])

            @pl.when((e >= E_W1) & (e < E_C))
            def _():
                j = e - E_W1
                start_pairs([(head_w(wuv_h, wuv_s, j, d, sem), out_w(wbo_h, wbo_s, j * 4 + d // 2, d % 2, sem))
                             for d in range(8)])

            @pl.when((e >= E_C) & (e < E_END))
            def _():
                j = e - E_C
                def one(b, d):
                    segs = pl.ds((d // 4) * 4, 4)
                    rb = (d // 2) % 2
                    cols = pl.ds((d % 2) * 256, 256)
                    return cp(c_h.at[b, segs, pl.ds(pl.multiple_of(j * 32 + rb * 16, 16), 16), cols],
                              c_s.at[b, j, segs, pl.ds(rb * 16, 16), cols], sem)
                start_pairs([(one(0, d), one(1, d)) for d in range(8)])

        def wait_extra(e):
            sem = sem_e.at[e & 3]

            @pl.when((e >= 0) & (e < E_W0))
            def _():
                rows_all(wo_s, pl.multiple_of((e - E_WO) * 128, 128), 128, sem).wait()

            @pl.when((e >= E_W0) & (e < E_W1))
            def _():
                head_w_all(wbq_s, e - E_W0, sem).wait()
                head_w_all(wuk_s, e - E_W0, sem).wait()

            @pl.when((e >= E_W1) & (e < E_C))
            def _():
                head_w_all(wuv_s, e - E_W1, sem).wait()
                rows_all(wbo_s, pl.multiple_of((e - E_W1) * 64, 64), 64, sem).wait()

            @pl.when((e >= E_C) & (e < E_END))
            def _():
                for b in range(NB):
                    v = c_s.at[b, e - E_C]
                    cp(v, v, sem).wait()

        def start_kv(k):
            slot = k & (NSG - 1)
            h0 = (k >> 6) * G
            r0 = (k & (NSTEP - 1)) * TR
            sem = sem_kv.at[slot]
            pairs = []
            for d in range(8):
                rows = pl.ds(pl.multiple_of(r0 + d * 16, 16), 16)
                pairs.append((cp(k_h.at[pl.ds(h0, G), rows, :], kv_s.at[slot, 0, :, pl.ds(d * 16, 16), :], sem),
                              cp(v_h.at[pl.ds(h0, G), rows, :], kv_s.at[slot, 1, :, pl.ds(d * 16, 16), :], sem)))
            start_pairs(pairs)

        def wait_kv(k):
            slot = k & (NSG - 1)
            cp(kv_s.at[slot], kv_s.at[slot], sem_kv.at[slot]).wait()

        row8 = lambda n: lax.broadcasted_iota(jnp.int32, (8, n), 0)

        def pad_rows(x2):
            r = row8(x2.shape[1])
            return jnp.where(r == 0, x2[0:1, :], jnp.where(r == 1, x2[1:2, :], 0.0))

        cp_xa = cp(xa_h, xa_s, sem_x.at[0])
        cp_xb = cp(xb_h, xb_s, sem_x.at[1])
        for j in range(L):
            start_q(j)
        cp_xa.start()
        cp_xb.start()
        for j in range(8):
            wait_q(j)
            if j + L < 8:
                start_q(j + L)
            else:
                start_kv(j + L - 8)
        cp_xa.wait()
        cp_xb.wait()

        if comp:
            with scope("T4"):
                xa8 = pad_rows(xa_s[...].astype(F32)).astype(BF)
                qa = jnp.zeros((8, H * DH), F32)
                for q in range(4):
                    qa = qa + jnp.dot(xa8[:, q * 128:(q + 1) * 128], wq_s[q], preferred_element_type=F32)
                r128 = row8(DH)
                for b in range(NB):
                    for gg in range(H // G):
                        blk = jnp.zeros((8, DH), F32)
                        for j in range(G):
                            h = gg * G + j
                            blk = jnp.where(r128 == j, qa[b:b + 1, h * DH:(h + 1) * DH], blk)
                        q_s[b * (H // G) + gg] = blk
            lat_s[...] = jnp.zeros(lat_s.shape, F32)
            lm_s[...] = jnp.full(lm_s.shape, -jnp.inf, F32)
            ll_s[...] = jnp.zeros(ll_s.shape, F32)
            lacc_s[...] = jnp.zeros(lacc_s.shape, F32)
            ob_s[...] = jnp.zeros(ob_s.shape, F32)
            oa_s[...] = jnp.zeros(oa_s.shape, F32)

        wbq32 = wbq_s.bitcast(U32)
        wuk32 = wuk_s.bitcast(U32)
        wuv32 = wuv_s.bitcast(U32)

        def head_pair(w32, jb, ii):
            base_row = pl.multiple_of(jb * 4, 4)
            blk = jnp.concatenate(
                [w32.at[q, pl.ds(base_row, 2036), :][pl.ds(ii, 128, stride=H // 2), :] for q in range(4)], axis=0)
            return _halves(blk)

        def per_pair(i, body):
            for ii in range(4):
                @pl.when((i & 3) == ii)
                def _():
                    body(i >> 2, ii)

        def t1_pair(jb, ii):
            with scope("T1"):
                xb8 = pad_rows(xb_s[...].astype(F32)).astype(BF)
                wq_pair = head_pair(wbq32, jb, ii)
                wk_pair = head_pair(wuk32, jb, ii)
                r512 = row8(DC)
                lat = [lat_s[b, jb] for b in range(NB)]
                for e in range(2):
                    q = jnp.dot(xb8, wq_pair[e], preferred_element_type=F32).astype(BF)
                    ql = lax.dot_general(q, wk_pair[e], NT, preferred_element_type=F32)
                    for b in range(NB):
                        lat[b] = jnp.where(r512 == 2 * ii + e, ql[b:b + 1, :], lat[b])
                for b in range(NB):
                    lat_s[b, jb] = lat[b]

        def t2(j):
            with scope("T2"):
                for b in range(NB):
                    ql = lat_s[b].reshape(H, DC).astype(BF)
                    cc = c_s[b, j].reshape(256, DC)
                    s = lax.dot_general(ql, cc, NT, preferred_element_type=F32)
                    m_old = lm_s[b]
                    m_new = jnp.maximum(m_old, jnp.max(s, axis=1, keepdims=True))
                    alpha = jnp.exp((m_old - m_new) * scale)
                    p = jnp.exp((s - m_new[:, 0:1]) * scale)
                    ll_s[b] = alpha * ll_s[b] + (p[:, 0:128] + p[:, 128:256])
                    lacc_s[b] = alpha[:, 0:1] * lacc_s[b] + jnp.dot(p.astype(BF), cc, preferred_element_type=F32)
                    lm_s[b] = m_new

        def t3_pair(jb, ii):
            with scope("T3"):
                wv_pair = head_pair(wuv32, jb, ii)
                r128 = row8(DH)
                rows = pl.ds(pl.multiple_of(jb * 8, 8), 8)
                lhs = [(lacc_s[b, rows, :] / jnp.sum(ll_s[b, rows, :], axis=1, keepdims=True)).astype(BF)
                       for b in range(NB)]
                for e in range(2):
                    hr = 2 * ii + e
                    wo_blk = wbo_s[jb, pl.ds(hr * DH, DH), :]
                    for b in range(NB):
                        ctx = jnp.dot(lhs[b], wv_pair[e], preferred_element_type=F32)
                        ctx = jnp.where(r128 == hr, ctx, 0.0).astype(BF)
                        ob_s[b] = ob_s[b] + jnp.dot(ctx, wo_blk, preferred_element_type=F32)

        r128 = row8(DH)

        def step(k, carry):
            m, l, acc = carry
            wait_kv(k)

            @pl.when(k + L < NK)
            def _():
                start_kv(k + L)

            @pl.when(((k & (EP - 1)) == 0) & (k < (P_T3 + 16 + EW) * EP))
            def _():
                e = k // EP
                ew = e - EW
                wait_extra(ew)
                start_extra(e)
                if comp:
                    if 't1' not in skip:
                        @pl.when((ew >= P_T1) & (ew < P_T1 + 16))
                        def _():
                            per_pair(ew - P_T1, t1_pair)
                    if 't2' not in skip:
                        @pl.when((ew >= E_C) & (ew < E_END))
                        def _():
                            t2(ew - E_C)
                    if 't3' not in skip:
                        @pl.when(ew >= P_T3)
                        def _():
                            per_pair(ew - P_T3, t3_pair)

            if not comp or 'a' in skip:
                return carry

            with scope("Astep"):
                slot = k & (NSG - 1)
                g = k >> 6
                first = (k & (NSTEP - 1)) == 0
                q = q_s[g].astype(BF)
                s = jnp.zeros((8, TR), F32)
                for j in range(G):
                    r = lax.dot_general(q, kv_s[slot, 0, j], NT, preferred_element_type=F32)
                    s = jnp.where(r128 == j, r, s)
                m_old = jnp.where(first, -jnp.inf, m)
                m_new = jnp.maximum(m_old, jnp.max(s, axis=1, keepdims=True))
                alpha = jnp.exp((m_old - m_new) * scale)
                p = jnp.exp((s - m_new) * scale)
                l = alpha * l + p
                pb = p.astype(BF)
                pv_ = jnp.zeros((8, DH), F32)
                for j in range(G):
                    r = jnp.dot(pb, kv_s[slot, 1, j], preferred_element_type=F32)
                    pv_ = jnp.where(r128 == j, r, pv_)
                acc = alpha * acc + pv_

            @pl.when((k & (NSTEP - 1)) == NSTEP - 1)
            def _():
                with scope("Afin"):
                    o = acc / jnp.sum(l, axis=1, keepdims=True)
                    b = g >> 2
                    res = oa_s[b]
                    for j in range(G):
                        oj = jnp.where(r128 == j, o, 0.0).astype(BF)
                        res = res + jnp.dot(oj, wo_s[g & 3, pl.ds(j * DH, DH), :], preferred_element_type=F32)
                    oa_s[b] = res
            return m_new, l, acc

        z = jnp.zeros((8, DH), F32)
        lax.fori_loop(0, NK, step, (z, z, z))

        if comp:
            for b in range(NB):
                out_ref[b:b + 1, 0:M] = jnp.sum(oa_s[b], axis=0, keepdims=True).astype(out_ref.dtype)
                out_ref[b:b + 1, M:2 * M] = jnp.sum(ob_s[b], axis=0, keepdims=True).astype(out_ref.dtype)
        else:
            out_ref[...] = jnp.zeros(out_ref.shape, out_ref.dtype)

    @jax.jit
    def fn(A_x, A_k_cache, A_v_cache, A_wq, A_wo, B_x, B_c_kv, B_w_q, B_w_uk, B_w_uv, B_w_o):
        args = (
            A_x.reshape(NB, M),
            A_k_cache.reshape(NB * H, S, DH),
            A_v_cache.reshape(NB * H, S, DH),
            A_wq.reshape(4, M // 4, H * DH),
            A_wo.reshape(4, H * DH // 4, M),
            B_x.reshape(NB, M),
            B_c_kv.reshape(NB, 8, S // 8, DC),
            B_w_q.reshape(4, M * H // 4, DH),
            B_w_uk.reshape(4, DC * H // 4, DH),
            B_w_uv.reshape(4, DC * H // 4, DH),
            B_w_o.reshape(4, H * DH // 4, M),
        )
        out = pl.pallas_call(
            kernel,
            in_specs=[pl.BlockSpec(memory_space=pl.ANY)] * 11,
            out_specs=pl.BlockSpec(memory_space=pltpu.VMEM),
            out_shape=jax.ShapeDtypeStruct((NB, 2 * M), BF),
            scratch_shapes=[
                pltpu.VMEM((NB, M), BF), pltpu.VMEM((NB, M), BF),
                pltpu.VMEM((4, M // 4, H * DH), BF), pltpu.VMEM((4, H * DH // 4, M), BF),
                pltpu.VMEM((NB, 32, 8, 32, DC), BF),
                pltpu.VMEM((4, M * H // 4, DH), BF), pltpu.VMEM((4, DC * H // 4, DH), BF), pltpu.VMEM((4, DC * H // 4, DH), BF),
                pltpu.VMEM((4, H * DH // 4, M), BF),
                pltpu.VMEM((NSG, 2, G, TR, DH), BF),
                pltpu.VMEM((NGRP, 8, DH), F32),
                pltpu.VMEM((NB, H // 8, 8, DC), F32),
                pltpu.VMEM((NB, H, 128), F32),
                pltpu.VMEM((NB, H, 128), F32),
                pltpu.VMEM((NB, H, DC), F32),
                pltpu.VMEM((NB, 8, M), F32),
                pltpu.VMEM((NB, 8, M), F32),
                pltpu.SemaphoreType.DMA((2,)),
                pltpu.SemaphoreType.DMA((8,)),
                pltpu.SemaphoreType.DMA((4,)),
                pltpu.SemaphoreType.DMA((NSG,)),
            ],
            compiler_params=pltpu.CompilerParams(vmem_limit_bytes=100 * 1024 * 1024, **cparams),
        )(*args)
        return out.reshape(NB, 1, 2 * M)
    return fn


_impl = make_kernel()


@jax.jit
def pallas_concat_heads__gqa_block_cached__compressed_kv_cla__decode_kernel(
    A_x: jax.Array,
    A_k_cache: jax.Array,
    A_v_cache: jax.Array,
    A_wq: jax.Array,
    A_wo: jax.Array,
    B_x: jax.Array,
    B_c_kv: jax.Array,
    B_w_q: jax.Array,
    B_w_uk: jax.Array,
    B_w_uv: jax.Array,
    B_w_o: jax.Array,
):
    return _impl(A_x, A_k_cache, A_v_cache, A_wq, A_wo,
                 B_x, B_c_kv, B_w_q, B_w_uk, B_w_uv, B_w_o)
```

```python
import jax
import jax.numpy as jnp
from jax import lax
import jax.experimental.pallas as pl
import jax.experimental.pallas.tpu as pltpu

BF = jnp.bfloat16
F32 = jnp.float32
U32 = jnp.uint32
NT = (((1,), (1,)), ((), ()))

NB, H, S, DH, M, DC = 2, 32, 8192, 128, 512, 512
SCALE = float(DH) ** -0.5

G = 8
SPH = 2
SEG = S // SPH
HPG = G // SPH
TR = 128
NSTEP = SEG // TR
LSTEP = NSTEP.bit_length() - 1
NGRP = NB * H // HPG
NK = NGRP * NSTEP
NSLOT = 8
LOOK = 7
EP = 4
EW = 2
E_W0, E_W1, E_C, E_END = 0, 16, 32, 64
P_T1, P_T3 = 16, 64
PRIO_A, PRIO_B = 1, 0


def _halves(w32):
    lo = pltpu.bitcast(w32 << 16, F32).astype(BF)
    hi = pltpu.bitcast(w32 & jnp.uint32(0xFFFF0000), F32).astype(BF)
    return lo, hi


def _rows(n):
    return lax.broadcasted_iota(jnp.int32, (8, n), 0)


def _pad_rows(x2):
    r = _rows(x2.shape[1])
    return jnp.where(r == 0, x2[0:1, :], jnp.where(r == 1, x2[1:2, :], 0.0))


def _kernel(xa_h, k_h, v_h, wq_h, wo_h, xb_h, c_h, wbq_h, wuk_h, wuv_h, wbo_h,
            out_ref,
            xa_s, xb_s, wq_s, wo_s, c_s, wbq_s, wuk_s, wuv_s, wbo_s,
            kv_s, q_s, lat_s, lm_s, ll_s, lacc_s, ob_s, oa_s, st_s,
            sem_x, sem_q, sem_e, sem_kv, sem_wo):
    cp = pltpu.make_async_copy

    def start_pairs(pairs):
        for a, b in pairs:
            a.start(priority=PRIO_A)
            b.start(priority=PRIO_B)

    def wait_all(view, sem):
        cp(view, view, sem).wait()

    def start_q(j):
        rows = pl.ds(j * 16, 16)
        lst = [cp(wq_h.at[sg, rows, pl.ds(d * 1024, 1024)], wq_s.at[sg, rows, pl.ds(d * 1024, 1024)],
                  sem_q.at[j]) for d in range(4) for sg in range(4)]
        start_pairs([(lst[2 * d], lst[2 * d + 1]) for d in range(8)])

    def wait_q(j):
        wait_all(wq_s.at[:, pl.ds(j * 16, 16), :], sem_q.at[j])

    def head_w(src, dst, j, d, sem):
        rows = pl.ds(pl.multiple_of((j * 8 + d) * 32, 32), 32)
        return cp(src.at[:, rows, :], dst.at[:, rows, :], sem)

    def head_w_view(dst, j):
        return dst.at[:, pl.ds(pl.multiple_of(j * 256, 256), 256), :]

    def out_w(j, d, sem):
        rows = pl.ds(pl.multiple_of((j * 4 + d // 2) * 16, 16), 16)
        cols = pl.ds((d % 2) * 256, 256)
        return cp(wbo_h.at[:, rows, cols], wbo_s.at[:, rows, cols], sem)

    def c_piece(b, j, d, sem):
        segs = pl.ds((d // 4) * 4, 4)
        rb = (d // 2) % 2
        cols = pl.ds((d % 2) * 256, 256)
        return cp(c_h.at[b, segs, pl.ds(pl.multiple_of(j * 32 + rb * 16, 16), 16), cols],
                  c_s.at[b, j, segs, pl.ds(rb * 16, 16), cols], sem)

    def start_extra(e):
        sem = sem_e.at[e & 3]

        @pl.when((e >= E_W0) & (e < E_W1))
        def _():
            j = e - E_W0
            start_pairs([(head_w(wbq_h, wbq_s, j, d, sem), head_w(wuk_h, wuk_s, j, d, sem))
                         for d in range(8)])

        @pl.when((e >= E_W1) & (e < E_C))
        def _():
            j = e - E_W1
            start_pairs([(head_w(wuv_h, wuv_s, j, d, sem), out_w(j, d, sem)) for d in range(8)])

        @pl.when((e >= E_C) & (e < E_END))
        def _():
            j = e - E_C
            start_pairs([(c_piece(0, j, d, sem), c_piece(1, j, d, sem)) for d in range(8)])

    def wait_extra(e):
        sem = sem_e.at[e & 3]

        @pl.when((e >= E_W0) & (e < E_W1))
        def _():
            wait_all(head_w_view(wbq_s, e - E_W0), sem)
            wait_all(head_w_view(wuk_s, e - E_W0), sem)

        @pl.when((e >= E_W1) & (e < E_C))
        def _():
            wait_all(head_w_view(wuv_s, e - E_W1), sem)
            wait_all(wbo_s.at[:, pl.ds(pl.multiple_of((e - E_W1) * 64, 64), 64), :], sem)

        @pl.when((e >= E_C) & (e < E_END))
        def _():
            for b in range(NB):
                wait_all(c_s.at[b, e - E_C], sem)

    def start_kv(k):
        slot = k & (NSLOT - 1)
        tg = k >> LSTEP
        seg0 = (((tg & 1) << 3) + (tg >> 1)) * G
        r0 = (k & (NSTEP - 1)) * TR
        sem = sem_kv.at[slot]
        pairs = []
        for d in range(8):
            rows = pl.ds(pl.multiple_of(r0 + d * 16, 16), 16)
            pairs.append((cp(k_h.at[pl.ds(seg0, G), rows, :], kv_s.at[slot, 0, :, pl.ds(d * 16, 16), :], sem),
                          cp(v_h.at[pl.ds(seg0, G), rows, :], kv_s.at[slot, 1, :, pl.ds(d * 16, 16), :], sem)))
        start_pairs(pairs)

    def wait_kv(k):
        slot = k & (NSLOT - 1)
        wait_all(kv_s.at[slot], sem_kv.at[slot])

    def start_wo(hq):
        lst = []
        for d in range(16):
            h = hq * HPG + d // 4
            rows = pl.ds((d % 4) * 32, 32)
            lst.append(cp(wo_h.at[h, rows, :], wo_s.at[h, rows, :], sem_wo.at[0]))
        start_pairs([(lst[d], lst[d + 8]) for d in range(8)])

    def wait_wo(hq):
        wait_all(wo_s.at[pl.ds(hq * HPG, HPG)], sem_wo.at[0])

    cp_xa = cp(xa_h, xa_s, sem_x.at[0])
    cp_xb = cp(xb_h, xb_s, sem_x.at[1])

    def start_pro(n):
        if n < 8:
            start_q(n)
        else:
            start_kv(n - 8)

    for n in range(LOOK):
        start_pro(n)
    cp_xa.start()
    cp_xb.start()
    for j in range(8):
        wait_q(j)
        start_pro(j + LOOK)
    cp_xa.wait()
    cp_xb.wait()

    r128 = _rows(DH)

    xa8 = _pad_rows(xa_s[...].astype(F32)).astype(BF)
    qa = jnp.zeros((8, H * DH), F32)
    for q in range(4):
        qa = qa + jnp.dot(xa8[:, q * 128:(q + 1) * 128], wq_s[q], preferred_element_type=F32)
    for b in range(NB):
        for gg in range(H // HPG):
            blk = jnp.zeros((8, DH), F32)
            for j in range(HPG):
                h = gg * HPG + j
                blk = jnp.where(r128 // SPH == j, qa[b:b + 1, h * DH:(h + 1) * DH], blk)
            q_s[b * (H // HPG) + gg] = blk

    lat_s[...] = jnp.zeros(lat_s.shape, F32)
    lm_s[...] = jnp.full(lm_s.shape, -jnp.inf, F32)
    ll_s[...] = jnp.zeros(ll_s.shape, F32)
    lacc_s[...] = jnp.zeros(lacc_s.shape, F32)
    ob_s[...] = jnp.zeros(ob_s.shape, F32)
    oa_s[...] = jnp.zeros(oa_s.shape, F32)

    wbq32 = wbq_s.bitcast(U32)
    wuk32 = wuk_s.bitcast(U32)
    wuv32 = wuv_s.bitcast(U32)

    def head_pair(w32, jb, ii):
        base = pl.multiple_of(jb * 4, 4)
        blk = jnp.concatenate(
            [w32.at[q, pl.ds(base, 2036), :][pl.ds(ii, 128, stride=H // 2), :] for q in range(4)],
            axis=0)
        return _halves(blk)

    def per_pair(i, body):
        for ii in range(4):
            @pl.when((i & 3) == ii)
            def _():
                body(i >> 2, ii)

    def latent_query(jb, ii):
        xb8 = _pad_rows(xb_s[...].astype(F32)).astype(BF)
        wq_pair = head_pair(wbq32, jb, ii)
        wk_pair = head_pair(wuk32, jb, ii)
        r512 = _rows(DC)
        lat = [lat_s[b, jb] for b in range(NB)]
        for e in range(2):
            q = jnp.dot(xb8, wq_pair[e], preferred_element_type=F32).astype(BF)
            ql = lax.dot_general(q, wk_pair[e], NT, preferred_element_type=F32)
            for b in range(NB):
                lat[b] = jnp.where(r512 == 2 * ii + e, ql[b:b + 1, :], lat[b])
        for b in range(NB):
            lat_s[b, jb] = lat[b]

    def latent_attend(j):
        for b in range(NB):
            ql = lat_s[b].reshape(H, DC).astype(BF)
            cc = c_s[b, j].reshape(256, DC)
            s = lax.dot_general(ql, cc, NT, preferred_element_type=F32)
            m_old = lm_s[b]
            m_new = jnp.maximum(m_old, jnp.max(s, axis=1, keepdims=True))
            alpha = jnp.exp((m_old - m_new) * SCALE)
            p = jnp.exp((s - m_new[:, 0:1]) * SCALE)
            ll_s[b] = alpha * ll_s[b] + (p[:, 0:128] + p[:, 128:256])
            lacc_s[b] = alpha[:, 0:1] * lacc_s[b] + jnp.dot(p.astype(BF), cc, preferred_element_type=F32)
            lm_s[b] = m_new

    def context_out(jb, ii):
        wv_pair = head_pair(wuv32, jb, ii)
        rows = pl.ds(pl.multiple_of(jb * 8, 8), 8)
        lhs = [(lacc_s[b, rows, :] / jnp.sum(ll_s[b, rows, :], axis=1, keepdims=True)).astype(BF)
               for b in range(NB)]
        for e in range(2):
            hr = 2 * ii + e
            wo_blk = wbo_s[jb, pl.ds(hr * DH, DH), :]
            for b in range(NB):
                ctx = jnp.dot(lhs[b], wv_pair[e], preferred_element_type=F32)
                ctx = jnp.where(r128 == hr, ctx, 0.0).astype(BF)
                ob_s[b] = ob_s[b] + jnp.dot(ctx, wo_blk, preferred_element_type=F32)

    def over_head(x, op):
        return op(x, jnp.where((r128 & 1) == 0, pltpu.roll(x, 7, 0), pltpu.roll(x, 1, 0)))

    def step(k, carry):
        m, l, acc = carry
        wait_kv(k)

        @pl.when(k + LOOK < NK)
        def _():
            start_kv(k + LOOK)

        @pl.when(((k + LOOK) & (2 * NSTEP - 1)) == 0)
        def _():
            start_wo(((k + LOOK) >> (LSTEP + 1)) - 1)

        @pl.when(((k & (EP - 1)) == 0) & (k < (P_T3 + 17 + EW) * EP))
        def _():
            e = k // EP
            ew = e - EW
            wait_extra(ew)
            start_extra(e)

            @pl.when((ew >= P_T1) & (ew < P_T1 + 16))
            def _():
                per_pair(ew - P_T1, latent_query)

            @pl.when((ew >= E_C) & (ew < E_END))
            def _():
                latent_attend(ew - E_C)

            @pl.when((ew >= P_T3) & (ew < P_T3 + 16))
            def _():
                per_pair(ew - P_T3, context_out)

            @pl.when(ew == P_T3 + 16)
            def _():
                for b in range(NB):
                    out_ref[b:b + 1, M:2 * M] = jnp.sum(ob_s[b], axis=0, keepdims=True).astype(out_ref.dtype)

        slot = k & (NSLOT - 1)
        tg = k >> LSTEP
        q = q_s[((tg & 1) << 3) + (tg >> 1)].astype(BF)
        s = jnp.zeros((8, TR), F32)
        for j in range(G):
            r = lax.dot_general(q, kv_s[slot, 0, j], NT, preferred_element_type=F32)
            s = jnp.where(r128 == j, r, s)
        m_old = jnp.where((k & (NSTEP - 1)) == 0, -jnp.inf, m)
        m_new = jnp.maximum(m_old, jnp.max(s, axis=1, keepdims=True))
        alpha = jnp.exp((m_old - m_new) * SCALE)
        p = jnp.exp((s - m_new) * SCALE)
        l = alpha * l + p
        pb = p.astype(BF)
        pv = jnp.zeros((8, DH), F32)
        for j in range(G):
            r = jnp.dot(pb, kv_s[slot, 1, j], preferred_element_type=F32)
            pv = jnp.where(r128 == j, r, pv)
        acc = alpha * acc + pv

        @pl.when((k & (NSTEP - 1)) == NSTEP - 1)
        def _():
            f = jnp.exp((m_new - over_head(m_new, jnp.maximum)) * SCALE)
            lsum = over_head(f * jnp.sum(l, axis=1, keepdims=True), jnp.add)
            o = over_head(f * acc, jnp.add) / lsum

            @pl.when((tg & 1) == 0)
            def _():
                st_s[...] = o

            @pl.when((tg & 1) == 1)
            def _():
                hq = tg >> 1
                both = jnp.where((r128 & 1) == 0, st_s[...], o)
                wait_wo(hq)
                res = oa_s[...]
                for j in range(HPG):
                    oj = jnp.where((r128 >> 1) == j, both, 0.0).astype(BF)
                    res = res + jnp.dot(oj, wo_s[hq * HPG + j], preferred_element_type=F32)
                oa_s[...] = res

        return m_new, l, acc

    z = jnp.zeros((8, DH), F32)
    lax.fori_loop(0, NK, step, (z, z, z))

    r512 = _rows(M)
    for b in range(NB):
        out_ref[b:b + 1, 0:M] = jnp.sum(jnp.where((r512 & 1) == b, oa_s[...], 0.0), axis=0,
                                        keepdims=True).astype(out_ref.dtype)


@jax.jit
def pallas_concat_heads__gqa_block_cached__compressed_kv_cla__decode_kernel(
    A_x: jax.Array,
    A_k_cache: jax.Array,
    A_v_cache: jax.Array,
    A_wq: jax.Array,
    A_wo: jax.Array,
    B_x: jax.Array,
    B_c_kv: jax.Array,
    B_w_q: jax.Array,
    B_w_uk: jax.Array,
    B_w_uv: jax.Array,
    B_w_o: jax.Array,
):
    args = (
        A_x.reshape(NB, M),
        A_k_cache.reshape(NB * H * SPH, SEG, DH),
        A_v_cache.reshape(NB * H * SPH, SEG, DH),
        A_wq.reshape(4, M // 4, H * DH),
        A_wo.reshape(H, DH, M),
        B_x.reshape(NB, M),
        B_c_kv.reshape(NB, 8, S // 8, DC),
        B_w_q.reshape(4, M * H // 4, DH),
        B_w_uk.reshape(4, DC * H // 4, DH),
        B_w_uv.reshape(4, DC * H // 4, DH),
        B_w_o.reshape(4, H * DH // 4, M),
    )
    out = pl.pallas_call(
        _kernel,
        in_specs=[pl.BlockSpec(memory_space=pl.ANY)] * 11,
        out_specs=pl.BlockSpec(memory_space=pltpu.VMEM),
        out_shape=jax.ShapeDtypeStruct((NB, 2 * M), BF),
        scratch_shapes=[
            pltpu.VMEM((NB, M), BF),
            pltpu.VMEM((NB, M), BF),
            pltpu.VMEM((4, M // 4, H * DH), BF),
            pltpu.VMEM((H, DH, M), BF),
            pltpu.VMEM((NB, 32, 8, 32, DC), BF),
            pltpu.VMEM((4, M * H // 4, DH), BF),
            pltpu.VMEM((4, DC * H // 4, DH), BF),
            pltpu.VMEM((4, DC * H // 4, DH), BF),
            pltpu.VMEM((4, H * DH // 4, M), BF),
            pltpu.VMEM((NSLOT, 2, G, TR, DH), BF),
            pltpu.VMEM((NGRP, 8, DH), F32),
            pltpu.VMEM((NB, H // 8, 8, DC), F32),
            pltpu.VMEM((NB, H, 128), F32),
            pltpu.VMEM((NB, H, 128), F32),
            pltpu.VMEM((NB, H, DC), F32),
            pltpu.VMEM((NB, 8, M), F32),
            pltpu.VMEM((8, M), F32),
            pltpu.VMEM((8, DH), F32),
            pltpu.SemaphoreType.DMA((2,)),
            pltpu.SemaphoreType.DMA((8,)),
            pltpu.SemaphoreType.DMA((4,)),
            pltpu.SemaphoreType.DMA((NSLOT,)),
            pltpu.SemaphoreType.DMA((1,)),
        ],
        compiler_params=pltpu.CompilerParams(
            vmem_limit_bytes=100 * 1024 * 1024,
            disable_bounds_checks=True,
            disable_semaphore_checks=True,
        ),
    )(*args)
    return out.reshape(NB, 1, 2 * M)
```

```python
import jax
import jax.numpy as jnp
from jax import lax
import jax.experimental.pallas as pl
import jax.experimental.pallas.tpu as pltpu

BF = jnp.bfloat16
F32 = jnp.float32
U32 = jnp.uint32
NT = (((1,), (1,)), ((), ()))

NB, H, S, DH, M, DC = 2, 32, 8192, 128, 512, 512
SCALE = float(DH) ** -0.5

G = 8
SPH = 2
SEG = S // SPH
HPG = G // SPH
TR = 128
NSTEP = SEG // TR
LSTEP = NSTEP.bit_length() - 1
NGRP = NB * H // HPG
NK = NGRP * NSTEP
NSLOT = 8
LOOK = 7
EP = 4
EW = 2
E_W0, E_W1, E_C, E_END = 0, 16, 32, 64
P_T1, P_T3 = 16, 64
PRIO_A, PRIO_B = 1, 0


def _halves(w32):
    lo = pltpu.bitcast(w32 << 16, F32).astype(BF)
    hi = pltpu.bitcast(w32 & jnp.uint32(0xFFFF0000), F32).astype(BF)
    return lo, hi


def _transpose8(a):
    r = lax.broadcasted_iota(jnp.int32, (8, DH), 0)
    a = list(a)
    for d in (4, 2, 1):
        low = (r & d) == 0
        for m in range(8):
            if m & d == 0:
                x, y = a[m], a[m + d]
                a[m] = jnp.where(low, x, pltpu.roll(y, d, 0))
                a[m + d] = jnp.where(low, pltpu.roll(x, 8 - d, 0), y)
    return a


def _rows(n):
    return lax.broadcasted_iota(jnp.int32, (8, n), 0)


def _pad_rows(x2):
    r = _rows(x2.shape[1])
    return jnp.where(r == 0, x2[0:1, :], jnp.where(r == 1, x2[1:2, :], 0.0))


def _kernel(xa_h, k_h, v_h, wq_h, wo_h, xb_h, c_h, wbq_h, wuk_h, wuv_h, wbo_h,
            out_ref,
            xa_s, xb_s, wq_s, wo_s, c_s, wbq_s, wuk_s, wuv_s, wbo_s,
            wdq_s, wdk_s, wdv_s,
            kv_s, q_s, lat_s, lm_s, ll_s, lacc_s, ob_s, oa_s, st_s,
            sem_x, sem_q, sem_e, sem_kv, sem_wo):
    cp = pltpu.make_async_copy

    def start_pairs(pairs):
        for a, b in pairs:
            a.start(priority=PRIO_A)
            b.start(priority=PRIO_B)

    def wait_all(view, sem):
        cp(view, view, sem).wait()

    def start_q(j):
        rows = pl.ds(j * 16, 16)
        lst = [cp(wq_h.at[sg, rows, pl.ds(d * 1024, 1024)], wq_s.at[sg, rows, pl.ds(d * 1024, 1024)],
                  sem_q.at[j]) for d in range(4) for sg in range(4)]
        start_pairs([(lst[2 * d], lst[2 * d + 1]) for d in range(8)])

    def wait_q(j):
        wait_all(wq_s.at[:, pl.ds(j * 16, 16), :], sem_q.at[j])

    def head_w(src, dst, j, d, sem):
        rows = pl.ds(pl.multiple_of((j * 8 + d) * 32, 32), 32)
        return cp(src.at[:, rows, :], dst.at[:, rows, :], sem)

    def head_w_view(dst, j):
        return dst.at[:, pl.ds(pl.multiple_of(j * 256, 256), 256), :]

    def out_w(j, d, sem):
        rows = pl.ds(pl.multiple_of((j * 4 + d // 2) * 16, 16), 16)
        cols = pl.ds((d % 2) * 256, 256)
        return cp(wbo_h.at[:, rows, cols], wbo_s.at[:, rows, cols], sem)

    def c_piece(b, j, d, sem):
        segs = pl.ds((d // 4) * 4, 4)
        rb = (d // 2) % 2
        cols = pl.ds((d % 2) * 256, 256)
        return cp(c_h.at[b, segs, pl.ds(pl.multiple_of(j * 32 + rb * 16, 16), 16), cols],
                  c_s.at[b, j, segs, pl.ds(rb * 16, 16), cols], sem)

    def start_extra(e):
        sem = sem_e.at[e & 3]

        @pl.when((e >= E_W0) & (e < E_W1))
        def _():
            j = e - E_W0
            start_pairs([(head_w(wbq_h, wbq_s, j, d, sem), head_w(wuk_h, wuk_s, j, d, sem))
                         for d in range(8)])

        @pl.when((e >= E_W1) & (e < E_C))
        def _():
            j = e - E_W1
            start_pairs([(head_w(wuv_h, wuv_s, j, d, sem), out_w(j, d, sem)) for d in range(8)])

        @pl.when((e >= E_C) & (e < E_END))
        def _():
            j = e - E_C
            start_pairs([(c_piece(0, j, d, sem), c_piece(1, j, d, sem)) for d in range(8)])

    def wait_extra(e):
        sem = sem_e.at[e & 3]

        @pl.when((e >= E_W0) & (e < E_W1))
        def _():
            wait_all(head_w_view(wbq_s, e - E_W0), sem)
            wait_all(head_w_view(wuk_s, e - E_W0), sem)

        @pl.when((e >= E_W1) & (e < E_C))
        def _():
            wait_all(head_w_view(wuv_s, e - E_W1), sem)
            wait_all(wbo_s.at[:, pl.ds(pl.multiple_of((e - E_W1) * 64, 64), 64), :], sem)

        @pl.when((e >= E_C) & (e < E_END))
        def _():
            for b in range(NB):
                wait_all(c_s.at[b, e - E_C], sem)

    def start_kv(k):
        slot = k & (NSLOT - 1)
        tg = k >> LSTEP
        seg0 = (((tg & 1) << 3) + (tg >> 1)) * G
        r0 = (k & (NSTEP - 1)) * TR
        sem = sem_kv.at[slot]
        pairs = []
        for d in range(8):
            rows = pl.ds(pl.multiple_of(r0 + d * 16, 16), 16)
            pairs.append((cp(k_h.at[pl.ds(seg0, G), rows, :], kv_s.at[slot, 0, :, pl.ds(d * 16, 16), :], sem),
                          cp(v_h.at[pl.ds(seg0, G), rows, :], kv_s.at[slot, 1, :, pl.ds(d * 16, 16), :], sem)))
        start_pairs(pairs)

    def wait_kv(k):
        slot = k & (NSLOT - 1)
        wait_all(kv_s.at[slot], sem_kv.at[slot])

    def start_wo(hq):
        lst = []
        for d in range(16):
            h = hq * HPG + d // 4
            rows = pl.ds((d % 4) * 32, 32)
            lst.append(cp(wo_h.at[h, rows, :], wo_s.at[h, rows, :], sem_wo.at[0]))
        start_pairs([(lst[d], lst[d + 8]) for d in range(8)])

    def wait_wo(hq):
        wait_all(wo_s.at[pl.ds(hq * HPG, HPG)], sem_wo.at[0])

    cp_xa = cp(xa_h, xa_s, sem_x.at[0])
    cp_xb = cp(xb_h, xb_s, sem_x.at[1])

    def start_pro(n):
        if n < 8:
            start_q(n)
        else:
            start_kv(n - 8)

    for n in range(LOOK):
        start_pro(n)
    cp_xa.start()
    cp_xb.start()
    for j in range(8):
        wait_q(j)
        start_pro(j + LOOK)
    cp_xa.wait()
    cp_xb.wait()

    r128 = _rows(DH)

    xa8 = _pad_rows(xa_s[...].astype(F32)).astype(BF)
    qa = jnp.zeros((8, H * DH), F32)
    for q in range(4):
        qa = qa + jnp.dot(xa8[:, q * 128:(q + 1) * 128], wq_s[q], preferred_element_type=F32)
    for b in range(NB):
        for gg in range(H // HPG):
            blk = jnp.zeros((8, DH), F32)
            for j in range(HPG):
                h = gg * HPG + j
                blk = jnp.where(r128 // SPH == j, qa[b:b + 1, h * DH:(h + 1) * DH], blk)
            q_s[b * (H // HPG) + gg] = blk

    lat_s[...] = jnp.zeros(lat_s.shape, F32)
    lm_s[...] = jnp.full(lm_s.shape, -jnp.inf, F32)
    ll_s[...] = jnp.zeros(ll_s.shape, F32)
    lacc_s[...] = jnp.zeros(lacc_s.shape, F32)
    ob_s[...] = jnp.zeros(ob_s.shape, F32)
    oa_s[...] = jnp.zeros(oa_s.shape, F32)

    def by_head_pair(src_s, dst_s, j):
        for q in range(4):
            x = pltpu.bitcast(src_s[q, pl.ds(pl.multiple_of(j * 256, 256), 256), :], U32)
            rows = pl.ds(pl.multiple_of(q * 128 + j * 8, 8), 8)
            for half in range(2):
                t = _transpose8([x[r * 16 + half * 8:r * 16 + half * 8 + 8, :] for r in range(8)])
                for i in range(8):
                    dst_s[half * 8 + i, rows, :] = t[i]

    def latent_query(i):
        xb8 = _pad_rows(xb_s[...].astype(F32)).astype(BF)
        wq_pair = _halves(wdq_s[i])
        wk_pair = _halves(wdk_s[i])
        jb = i >> 2
        r512 = _rows(DC)
        lat = [lat_s[b, jb] for b in range(NB)]
        for e in range(2):
            q = jnp.dot(xb8, wq_pair[e], preferred_element_type=F32).astype(BF)
            ql = lax.dot_general(q, wk_pair[e], NT, preferred_element_type=F32)
            for b in range(NB):
                lat[b] = jnp.where(r512 == ((2 * i + e) & 7), ql[b:b + 1, :], lat[b])
        for b in range(NB):
            lat_s[b, jb] = lat[b]

    def latent_attend(j):
        for b in range(NB):
            ql = lat_s[b].reshape(H, DC).astype(BF)
            cc = c_s[b, j].reshape(256, DC)
            s = lax.dot_general(ql, cc, NT, preferred_element_type=F32)
            m_old = lm_s[b]
            m_new = jnp.maximum(m_old, jnp.max(s, axis=1, keepdims=True))
            alpha = jnp.exp((m_old - m_new) * SCALE)
            p = jnp.exp((s - m_new[:, 0:1]) * SCALE)
            ll_s[b] = alpha * ll_s[b] + (p[:, 0:128] + p[:, 128:256])
            lacc_s[b] = alpha[:, 0:1] * lacc_s[b] + jnp.dot(p.astype(BF), cc, preferred_element_type=F32)
            lm_s[b] = m_new

    def context_out(i):
        wv_pair = _halves(wdv_s[i])
        jb = i >> 2
        rows = pl.ds(pl.multiple_of(jb * 8, 8), 8)
        lhs = [(lacc_s[b, rows, :] / jnp.sum(ll_s[b, rows, :], axis=1, keepdims=True)).astype(BF)
               for b in range(NB)]
        for e in range(2):
            hr = (2 * i + e) & 7
            wo_blk = wbo_s[jb, pl.ds(pl.multiple_of(hr * DH, DH), DH), :]
            for b in range(NB):
                ctx = jnp.dot(lhs[b], wv_pair[e], preferred_element_type=F32)
                ctx = jnp.where(r128 == hr, ctx, 0.0).astype(BF)
                ob_s[b] = ob_s[b] + jnp.dot(ctx, wo_blk, preferred_element_type=F32)

    def over_head(x, op):
        return op(x, jnp.where((r128 & 1) == 0, pltpu.roll(x, 7, 0), pltpu.roll(x, 1, 0)))

    def step(k, carry):
        m, l, acc = carry
        wait_kv(k)

        @pl.when(k + LOOK < NK)
        def _():
            start_kv(k + LOOK)

        @pl.when(((k + LOOK) & (2 * NSTEP - 1)) == 0)
        def _():
            start_wo(((k + LOOK) >> (LSTEP + 1)) - 1)

        @pl.when(((k & (EP - 1)) == 0) & (k < (P_T3 + 17 + EW) * EP))
        def _():
            e = k // EP
            ew = e - EW
            wait_extra(ew)
            start_extra(e)

            @pl.when((ew >= E_W0) & (ew < E_W1))
            def _():
                by_head_pair(wbq_s, wdq_s, ew - E_W0)
                by_head_pair(wuk_s, wdk_s, ew - E_W0)

            @pl.when((ew >= E_W1) & (ew < E_C))
            def _():
                by_head_pair(wuv_s, wdv_s, ew - E_W1)

            @pl.when((ew >= P_T1) & (ew < P_T1 + 16))
            def _():
                latent_query(ew - P_T1)

            @pl.when((ew >= E_C) & (ew < E_END))
            def _():
                latent_attend(ew - E_C)

            @pl.when((ew >= P_T3) & (ew < P_T3 + 16))
            def _():
                context_out(ew - P_T3)

            @pl.when(ew == P_T3 + 16)
            def _():
                for b in range(NB):
                    out_ref[b:b + 1, M:2 * M] = jnp.sum(ob_s[b], axis=0, keepdims=True).astype(out_ref.dtype)

        slot = k & (NSLOT - 1)
        tg = k >> LSTEP
        q = q_s[((tg & 1) << 3) + (tg >> 1)].astype(BF)
        s = jnp.zeros((8, TR), F32)
        for j in range(G):
            r = lax.dot_general(q, kv_s[slot, 0, j], NT, preferred_element_type=F32)
            s = jnp.where(r128 == j, r, s)
        m_old = jnp.where((k & (NSTEP - 1)) == 0, -jnp.inf, m)
        m_new = jnp.maximum(m_old, jnp.max(s, axis=1, keepdims=True))
        alpha = jnp.exp((m_old - m_new) * SCALE)
        p = jnp.exp((s - m_new) * SCALE)
        l = alpha * l + p
        pb = p.astype(BF)
        pv = jnp.zeros((8, DH), F32)
        for j in range(G):
            r = jnp.dot(pb, kv_s[slot, 1, j], preferred_element_type=F32)
            pv = jnp.where(r128 == j, r, pv)
        acc = alpha * acc + pv

        @pl.when((k & (NSTEP - 1)) == NSTEP - 1)
        def _():
            f = jnp.exp((m_new - over_head(m_new, jnp.maximum)) * SCALE)
            lsum = over_head(f * jnp.sum(l, axis=1, keepdims=True), jnp.add)
            o = over_head(f * acc, jnp.add) / lsum

            @pl.when((tg & 1) == 0)
            def _():
                st_s[...] = o

            @pl.when((tg & 1) == 1)
            def _():
                hq = tg >> 1
                both = jnp.where((r128 & 1) == 0, st_s[...], o)
                wait_wo(hq)
                res = oa_s[...]
                for j in range(HPG):
                    oj = jnp.where((r128 >> 1) == j, both, 0.0).astype(BF)
                    res = res + jnp.dot(oj, wo_s[hq * HPG + j], preferred_element_type=F32)
                oa_s[...] = res

        return m_new, l, acc

    z = jnp.zeros((8, DH), F32)
    lax.fori_loop(0, NK, step, (z, z, z))

    r512 = _rows(M)
    for b in range(NB):
        out_ref[b:b + 1, 0:M] = jnp.sum(jnp.where((r512 & 1) == b, oa_s[...], 0.0), axis=0,
                                        keepdims=True).astype(out_ref.dtype)


@jax.jit
def pallas_concat_heads__gqa_block_cached__compressed_kv_cla__decode_kernel(
    A_x: jax.Array,
    A_k_cache: jax.Array,
    A_v_cache: jax.Array,
    A_wq: jax.Array,
    A_wo: jax.Array,
    B_x: jax.Array,
    B_c_kv: jax.Array,
    B_w_q: jax.Array,
    B_w_uk: jax.Array,
    B_w_uv: jax.Array,
    B_w_o: jax.Array,
):
    args = (
        A_x.reshape(NB, M),
        A_k_cache.reshape(NB * H * SPH, SEG, DH),
        A_v_cache.reshape(NB * H * SPH, SEG, DH),
        A_wq.reshape(4, M // 4, H * DH),
        A_wo.reshape(H, DH, M),
        B_x.reshape(NB, M),
        B_c_kv.reshape(NB, 8, S // 8, DC),
        B_w_q.reshape(4, M * H // 4, DH),
        B_w_uk.reshape(4, DC * H // 4, DH),
        B_w_uv.reshape(4, DC * H // 4, DH),
        B_w_o.reshape(4, H * DH // 4, M),
    )
    out = pl.pallas_call(
        _kernel,
        in_specs=[pl.BlockSpec(memory_space=pl.ANY)] * 11,
        out_specs=pl.BlockSpec(memory_space=pltpu.VMEM),
        out_shape=jax.ShapeDtypeStruct((NB, 2 * M), BF),
        scratch_shapes=[
            pltpu.VMEM((NB, M), BF),
            pltpu.VMEM((NB, M), BF),
            pltpu.VMEM((4, M // 4, H * DH), BF),
            pltpu.VMEM((H, DH, M), BF),
            pltpu.VMEM((NB, 32, 8, 32, DC), BF),
            pltpu.VMEM((4, M * H // 4, DH), BF),
            pltpu.VMEM((4, DC * H // 4, DH), BF),
            pltpu.VMEM((4, DC * H // 4, DH), BF),
            pltpu.VMEM((4, H * DH // 4, M), BF),
            pltpu.VMEM((H // 2, M, DH), U32),
            pltpu.VMEM((H // 2, DC, DH), U32),
            pltpu.VMEM((H // 2, DC, DH), U32),
            pltpu.VMEM((NSLOT, 2, G, TR, DH), BF),
            pltpu.VMEM((NGRP, 8, DH), F32),
            pltpu.VMEM((NB, H // 8, 8, DC), F32),
            pltpu.VMEM((NB, H, 128), F32),
            pltpu.VMEM((NB, H, 128), F32),
            pltpu.VMEM((NB, H, DC), F32),
            pltpu.VMEM((NB, 8, M), F32),
            pltpu.VMEM((8, M), F32),
            pltpu.VMEM((8, DH), F32),
            pltpu.SemaphoreType.DMA((2,)),
            pltpu.SemaphoreType.DMA((8,)),
            pltpu.SemaphoreType.DMA((4,)),
            pltpu.SemaphoreType.DMA((NSLOT,)),
            pltpu.SemaphoreType.DMA((1,)),
        ],
        compiler_params=pltpu.CompilerParams(
            vmem_limit_bytes=100 * 1024 * 1024,
            disable_bounds_checks=True,
            disable_semaphore_checks=True,
        ),
    )(*args)
    return out.reshape(NB, 1, 2 * M)
```
